```python
import os as _os
_os.environ.setdefault("JAX_PLATFORMS", "cpu")
import jax
import jax.numpy as jnp

def _softmax(x, axis=-1):
    return jax.nn.softmax(x, axis=axis)
def _gelu(x):
    return jax.nn.gelu(x, approximate=True)
def _silu(x):
    return jax.nn.silu(x)
def _sigmoid(x):
    return jax.nn.sigmoid(x)
def _layernorm(x, axis=-1, eps=1e-5):
    m = jnp.mean(x, axis=axis, keepdims=True)
    v = jnp.var(x, axis=axis, keepdims=True)
    return (x - m) / jnp.sqrt(v + eps)
def _scatter_add(tgt, idx, src, axis=0):
    return tgt.at[idx].add(src)
def _segment_sum(src, seg, n):
    return jax.ops.segment_sum(src, seg, n)
class _Rng:
    def __init__(self, key):
        self._k = key
    def _next(self):
        self._k, sub = jax.random.split(self._k)
        return sub
    def normal(self, shape):
        return jax.random.normal(self._next(), shape, dtype=jnp.bfloat16)
    def randint(self, lo, hi, shape):
        return jax.random.randint(self._next(), shape, lo, hi, dtype=jnp.int32)
    def uniform(self, shape, lo=0.0, hi=1.0):
        return jax.random.uniform(self._next(), shape, jnp.bfloat16, lo, hi)
    def permutation(self, n):
        return jax.random.permutation(self._next(), n)


kernel_name = 'interleave_layers__grouped_kv_mqa__dense_activation_relu__prompt'

def setup_inputs():
    _rng = _Rng(jax.random.key(int.from_bytes(__import__("os").urandom(4), "little")))
    _w = (lambda a: (lambda t: t.astype(jnp.bfloat16) if jnp.issubdtype(t.dtype, jnp.floating) else t)(jnp.asarray(a)))
    def _A_setup():
        B, S, D, H = 1, 2048, 448, 16
        Dh = D // H
        return {
            "x": _w((lambda *s: _rng.normal(s) * 0.05)(B, S, D)),
            "wq": _w((lambda *s: _rng.normal(s) * 0.05)(D, H * Dh)),
            "wk": _w((lambda *s: _rng.normal(s) * 0.05)(D, Dh)),
            "wv": _w((lambda *s: _rng.normal(s) * 0.05)(D, Dh)),
            "wo": _w((lambda *s: _rng.normal(s) * 0.05)(H * Dh, D)),
        }
    _A_in = _A_setup()

    def _B_setup():
        B, S, D, Dff = 1, 2048, 448, 1792
        return {
            "x": _w((lambda *s: _rng.normal(s) * 0.05)(B, S, D)),
            "w1": _w((lambda *s: _rng.normal(s) * 0.05)(D, Dff)),
            "w2": _w((lambda *s: _rng.normal(s) * 0.05)(Dff, D)),
        }
    _B_in = _B_setup()

    return {
        "A_x": _A_in["x"],
        "A_wq": _A_in["wq"],
        "A_wk": _A_in["wk"],
        "A_wv": _A_in["wv"],
        "A_wo": _A_in["wo"],
        "B_x": _B_in["x"],
        "B_w1": _B_in["w1"],
        "B_w2": _B_in["w2"],
    }

def reference(A_x, A_wq, A_wk, A_wv, A_wo, B_x, B_w1, B_w2):
    def _A_ref(x, wq, wk, wv, wo):
        B, S, D = x.shape
        H = 16
        Dh = D // H
        q = (lambda x, *d: x.transpose(*d))((x @ wq).reshape(B, S, H, Dh), 0, 2, 1, 3)
        k = x @ wk
        v = x @ wv
        scores = jnp.einsum("bhqd,bkd->bhqk", q, k) * (Dh ** -0.5)
        p = _softmax(scores, axis=-1)
        o = jnp.einsum("bhqk,bkd->bhqd", p, v)
        return (lambda x, *d: x.transpose(*d))(o, 0, 2, 1, 3).reshape(B, S, H * Dh) @ wo

    def _B_ref(x, w1, w2):
        h = jnp.einsum("bsd,df->bsf", x, w1)
        zero = jnp.zeros_like(h)
        h = jnp.maximum(h, zero)
        return jnp.einsum("bsf,fd->bsd", h, w2)

    x = A_x
    x = x + _A_ref(_layernorm(x, axis=-1), A_wq, A_wk, A_wv, A_wo)
    x = x + _B_ref(_layernorm(x, axis=-1), B_w1, B_w2)
    x = x + _A_ref(_layernorm(x, axis=-1), A_wq, A_wk, A_wv, A_wo)
    x = x + _B_ref(_layernorm(x, axis=-1), B_w1, B_w2)
    return x
```

```python
import functools

import jax
import jax.numpy as jnp
import jax.experimental.pallas as pl
import jax.experimental.pallas.tpu as pltpu

F32 = jnp.float32
BF16 = jnp.bfloat16

S = 2048
D = 448
H = 16
DH = 28
HP = 32
DFF = 1792
TQ = 512
NQB = S // TQ
CK = 128
NC = S // CK
U = 4
SKEW = 3
FC = 256
EPS = 1e-5
QSCALE = (DH ** -0.5) * 1.4426950408889634


def _ln(x):
    m = jnp.mean(x, axis=0, keepdims=True)
    xc = x - m
    v = jnp.mean(xc * xc, axis=0, keepdims=True)
    return xc * jax.lax.rsqrt(v + EPS)


def _kernel(x_hbm, wq_hbm, wk_hbm, wv_hbm, wo_hbm, w1_hbm, w2_hbm, out_hbm,
            xin_ref, wq_ref, wk_ref, wv_ref, wo_ref, w1_ref,
            wqkvT_ref, woT_ref, w1T_ref, w2T_ref, tmp_ref,
            xT_ref, qT_ref, k_ref, vT_ref, oT_ref, s_ref, obuf_ref,
            sem_in, sem_out):
    def xcopy(b):
        return pltpu.make_async_copy(x_hbm.at[0, :, pl.ds(b * TQ, TQ)], xin_ref.at[b], sem_in.at[b])
    wcopies = [pltpu.make_async_copy(src, dst, sem_in.at[NQB + i])
               for i, (src, dst) in enumerate([(wq_hbm, wq_ref), (wk_hbm, wk_ref), (wv_hbm, wv_ref),
                                               (wo_hbm, wo_ref), (w1_hbm, w1_ref), (w2_hbm, w2T_ref)])]
    for i in range(3):
        wcopies[i].start()
    for b in range(NQB):
        xcopy(b).start()
    for i in range(3, 6):
        wcopies[i].start()

    wcopies[0].wait(); wcopies[1].wait(); wcopies[2].wait()
    wqkvT_ref[...] = jnp.zeros(wqkvT_ref.shape, wqkvT_ref.dtype)
    tmp_ref[0:D, :] = wq_ref[...].astype(F32).T
    for h in range(H):
        wqkvT_ref[h * HP:h * HP + DH, :] = tmp_ref[h * DH:(h + 1) * DH, :]
    wqkvT_ref[H * HP:H * HP + DH, :] = wk_ref[...].astype(F32)
    wqkvT_ref[(H + 1) * HP:(H + 1) * HP + DH, :] = wv_ref[...].astype(F32)

    for b in range(NQB):
        xcopy(b).wait()
        xT_ref[b] = xin_ref[b].astype(F32)

    def proj_phase():
        wT = wqkvT_ref[...].astype(BF16)
        def body(b, c):
            xn = _ln(xT_ref[b]).astype(BF16)
            qkv = jnp.dot(wT, xn, preferred_element_type=F32)
            qT_ref[b] = (qkv[0:H * HP] * QSCALE).astype(BF16)
            k_ref[pl.ds(pl.multiple_of(b * TQ, TQ), TQ), :] = qkv[H * HP:(H + 1) * HP].T.astype(BF16)
            v = qkv[(H + 1) * HP:(H + 2) * HP]
            row = jax.lax.broadcasted_iota(jnp.int32, v.shape, 0)
            vT_ref[b] = jnp.where(row == DH, 1.0, v).astype(BF16)
            return c
        jax.lax.fori_loop(0, NQB, body, 0)

    def s1_chunk(u, c, slot, m8):
        h = u & 15; qb = u >> 4
        if isinstance(u, int):
            qblk = qT_ref[qb, h * HP:(h + 1) * HP, :]
        else:
            qblk = qT_ref[qb, pl.ds(pl.multiple_of(h * HP, HP), HP), :]
        kblk = k_ref[c * CK:(c + 1) * CK, :]
        s = jnp.dot(kblk, qblk, preferred_element_type=F32)
        s_ref[slot * CK:(slot + 1) * CK, :] = s
        mm = jnp.max(s.reshape(CK // 8, 8, TQ), axis=0)
        return mm if m8 is None else jnp.maximum(m8, mm)

    def s2_chunk(c, slot, m, acc):
        p = jnp.exp2(s_ref[slot * CK:(slot + 1) * CK, :] - m).astype(BF16)
        per = TQ // CK
        vblk = vT_ref[c // per, :, (c % per) * CK:(c % per + 1) * CK]
        o = jnp.dot(vblk, p, preferred_element_type=F32)
        return o if acc is None else acc + o

    def finish(u, acc):
        h = u & 15; qb = u >> 4
        o = (acc * (1.0 / acc[DH:DH + 1, :])).astype(BF16)
        if isinstance(u, int):
            oT_ref[qb, h * HP:(h + 1) * HP, :] = o
        else:
            oT_ref[qb, pl.ds(pl.multiple_of(h * HP, HP), HP), :] = o

    RS = 2 * NC
    L = NC + SKEW
    B = U * NC
    NU = H * NQB
    NB = NU // U

    def attn_block(u0, m_cur, m8, last):
        ms = {0: m_cur}
        acc = None
        for i in range(B):
            gi = L + i
            su, sc = gi // NC, gi % NC
            if not (last and su >= U):
                m8 = s1_chunk(u0 + su, sc, gi % RS, m8 if sc > 0 else None)
                if sc == NC - 1:
                    ms[su] = jnp.max(m8, axis=0, keepdims=True)
            pu, pc = i // NC, i % NC
            acc = s2_chunk(pc, i % RS, ms[pu], acc if pc > 0 else None)
            if pc == NC - 1:
                finish(u0 + pu, acc)
        if last:
            return None
        return ms[U], m8

    def attn_phase():
        m8 = None
        m0 = None
        for gi in range(L):
            su, sc = gi // NC, gi % NC
            m8 = s1_chunk(su, sc, gi % RS, m8 if sc > 0 else None)
            if sc == NC - 1:
                m0 = jnp.max(m8, axis=0, keepdims=True)
        c = jax.lax.fori_loop(0, NB - 1, lambda t, c: attn_block(t * U, c[0], c[1], False), (m0, m8))
        attn_block((NB - 1) * U, c[0], c[1], True)

    def ffn_phase():
        def body(b, c):
            a = jnp.dot(woT_ref[...], oT_ref[b], preferred_element_type=F32)
            x1 = xT_ref[b] + a
            xn = _ln(x1).astype(BF16)
            y = x1
            for f in range(DFF // FC):
                hc = jnp.dot(w1T_ref[f * FC:(f + 1) * FC, :], xn, preferred_element_type=F32)
                hc = jnp.maximum(hc, 0.0).astype(BF16)
                y = y + jnp.dot(w2T_ref[:, f * FC:(f + 1) * FC], hc, preferred_element_type=F32)
            xT_ref[b] = y
            return c
        jax.lax.fori_loop(0, NQB, body, 0)

    def layer(l, c):
        proj_phase()

        @pl.when(l == 0)
        def _():
            wcopies[3].wait(); wcopies[4].wait(); wcopies[5].wait()
            tmp_ref[...] = jnp.zeros(tmp_ref.shape, F32)
            wo32 = wo_ref[...].astype(F32)
            for h in range(H):
                tmp_ref[h * HP:h * HP + DH, :] = wo32[h * DH:(h + 1) * DH, :]
            woT_ref[...] = tmp_ref[...].T.astype(BF16)
            w1T_ref[...] = w1_ref[...].T

        attn_phase()
        ffn_phase()
        return c
    jax.lax.fori_loop(0, 2, layer, 0)

    def ocopy(b):
        return pltpu.make_async_copy(obuf_ref.at[b], out_hbm.at[0, :, pl.ds(b * TQ, TQ)], sem_out.at[b])
    for b in range(NQB):
        obuf_ref[b] = xT_ref[b].astype(BF16)
        ocopy(b).start()
    for b in range(NQB):
        ocopy(b).wait()


@jax.jit
def pallas_interleave_layers__grouped_kv_mqa__dense_activation_relu__prompt_kernel(A_x, A_wq, A_wk, A_wv, A_wo, B_x, B_w1, B_w2):
    any_spec = pl.BlockSpec(memory_space=pltpu.HBM)
    scratch = [
        pltpu.VMEM((NQB, D, TQ), BF16),
        pltpu.VMEM((D, D), BF16),
        pltpu.VMEM((DH, D), BF16),
        pltpu.VMEM((DH, D), BF16),
        pltpu.VMEM((D, D), BF16),
        pltpu.VMEM((D, DFF), BF16),
        pltpu.VMEM(((H + 2) * HP, D), F32),
        pltpu.VMEM((D, H * HP), BF16),
        pltpu.VMEM((DFF, D), BF16),
        pltpu.VMEM((D, DFF), BF16),
        pltpu.VMEM((H * HP, D), F32),
        pltpu.VMEM((NQB, D, TQ), F32),
        pltpu.VMEM((NQB, H * HP, TQ), BF16),
        pltpu.VMEM((S, HP), BF16),
        pltpu.VMEM((NQB, HP, TQ), BF16),
        pltpu.VMEM((NQB, H * HP, TQ), BF16),
        pltpu.VMEM((2 * S, TQ), F32),
        pltpu.VMEM((NQB, D, TQ), BF16),
        pltpu.SemaphoreType.DMA((NQB + 6,)),
        pltpu.SemaphoreType.DMA((NQB,)),
    ]
    outT = pl.pallas_call(
        _kernel,
        out_shape=jax.ShapeDtypeStruct((1, D, S), BF16),
        in_specs=[any_spec] * 7,
        out_specs=any_spec,
        scratch_shapes=scratch,
        compiler_params=pltpu.CompilerParams(vmem_limit_bytes=100 * 1024 * 1024),
    )(jnp.transpose(A_x, (0, 2, 1)), A_wq, A_wk.T, A_wv.T, A_wo, B_w1, B_w2.T)
    return jnp.transpose(outT, (0, 2, 1))
```

```python
import functools

import jax
import jax.numpy as jnp
import jax.experimental.pallas as pl
import jax.experimental.pallas.tpu as pltpu

F32 = jnp.float32
BF16 = jnp.bfloat16

S = 2048
D = 448
H = 16
DH = 28
HP = 32
DFF = 1792
TQ = 512
NQB = S // TQ
CK = 128
NC = S // CK
U = 6
UL = 4
ORDER = 1
SKEW = 3
FC = 256
EPS = 1e-5
KROW = D
VROW = D + HP
QKVR = D + 2 * HP
QSCALE = (DH ** -0.5) * 1.4426950408889634


def _ln(x):
    m = jnp.mean(x, axis=0, keepdims=True)
    xc = x - m
    v = jnp.mean(xc * xc, axis=0, keepdims=True)
    return xc * jax.lax.rsqrt(v + EPS)


def _kernel(x_hbm, wq_hbm, wk_hbm, wv_hbm, wo_hbm, w1_hbm, w2_hbm, out_hbm,
            xin_ref, wq_ref, wk_ref, wv_ref, wo_ref, w1_ref,
            wqkvT_ref, woT_ref, w1T_ref, w2T_ref, tmp_ref,
            xT_ref, qT_ref, k_ref, vT_ref, oT_ref, s_ref, obuf_ref,
            sem_in, sem_out):
    def xcopy(b):
        off = b * TQ if isinstance(b, int) else pl.multiple_of(b * TQ, TQ)
        return pltpu.make_async_copy(x_hbm.at[0, :, pl.ds(off, TQ)], xin_ref.at[b], sem_in.at[b])
    wcopies = [pltpu.make_async_copy(src, dst, sem_in.at[NQB + i])
               for i, (src, dst) in enumerate([(wq_hbm, wq_ref), (wk_hbm, wk_ref), (wv_hbm, wv_ref),
                                               (wo_hbm, wo_ref), (w1_hbm, w1_ref), (w2_hbm, w2T_ref)])]
    for i in range(3):
        wcopies[i].start()
    for b in range(NQB):
        xcopy(b).start()
    for i in range(3, 6):
        wcopies[i].start()

    def proj_mm(b, xn):
        qkv = jnp.dot(wqkvT_ref[...], xn, preferred_element_type=F32)
        q = jnp.concatenate([qkv[h * DH:h * DH + HP] for h in range(H)], axis=0)
        qT_ref[b] = (q * QSCALE).astype(BF16)
        kT = qkv[KROW:KROW + HP].T.astype(BF16)
        if isinstance(b, int):
            k_ref[b * TQ:(b + 1) * TQ, :] = kT
        else:
            k_ref[pl.ds(pl.multiple_of(b * TQ, TQ), TQ), :] = kT
        v = qkv[VROW:VROW + HP]
        row = jax.lax.broadcasted_iota(jnp.int32, v.shape, 0)
        vT_ref[b] = jnp.where(row == DH, 1.0, v).astype(BF16)

    def proj(b, x):
        proj_mm(b, _ln(x).astype(BF16))

    wcopies[0].wait(); wcopies[1].wait(); wcopies[2].wait()
    wqkvT_ref[0:D, :] = wq_ref[...].T
    kv = jnp.concatenate([wk_ref[...].astype(F32), jnp.zeros((HP - DH, D), F32),
                          wv_ref[...].astype(F32), jnp.zeros((HP - DH, D), F32)], axis=0)
    wqkvT_ref[KROW:KROW + 2 * HP, :] = kv.astype(BF16)

    def proj0(b, c):
        xcopy(b).wait()
        x = xin_ref[b].astype(F32)
        xT_ref[b] = x
        proj(b, x)
        return c
    jax.lax.fori_loop(0, NQB - 1, proj0, 0)
    b = NQB - 1
    xcopy(b).wait()
    wcopies[3].wait(); wcopies[4].wait()
    x = xin_ref[b].astype(F32)
    xT_ref[b] = x
    proj(b, x)
    tmp_ref[...] = jnp.zeros((H * HP, D), F32)
    wo32 = wo_ref[...].astype(F32)
    for h in range(H):
        tmp_ref[h * HP:h * HP + DH, :] = wo32[h * DH:(h + 1) * DH, :]
    woT_ref[...] = tmp_ref[...].T.astype(BF16)
    w1T_ref[...] = w1_ref[...].T

    def s1_chunk(u, c, slot, m8):
        h = u & 15; qb = u >> 4
        if isinstance(u, int):
            qblk = qT_ref[qb, h * HP:(h + 1) * HP, :]
        else:
            qblk = qT_ref[qb, pl.ds(pl.multiple_of(h * HP, HP), HP), :]
        kblk = k_ref[c * CK:(c + 1) * CK, :]
        s = jnp.dot(kblk, qblk, preferred_element_type=F32)
        s_ref[slot * CK:(slot + 1) * CK, :] = s
        mm = jnp.max(s.reshape(CK // 8, 8, TQ), axis=0)
        return mm if m8 is None else jnp.maximum(m8, mm)

    def s2_chunk(c, slot, m, acc):
        p = jnp.exp2(s_ref[slot * CK:(slot + 1) * CK, :] - m).astype(BF16)
        per = TQ // CK
        vblk = vT_ref[c // per, :, (c % per) * CK:(c % per + 1) * CK]
        o = jnp.dot(vblk, p, preferred_element_type=F32)
        return o if acc is None else acc + o

    def finish(u, acc):
        h = u & 15; qb = u >> 4
        o = (acc * (1.0 / acc[DH:DH + 1, :])).astype(BF16)
        if isinstance(u, int):
            oT_ref[qb, h * HP:(h + 1) * HP, :] = o
        else:
            oT_ref[qb, pl.ds(pl.multiple_of(h * HP, HP), HP), :] = o

    RS = 2 * NC
    L = NC + SKEW
    NU = H * NQB
    NI = (NU - UL) // U
    assert U * NI + UL == NU and U % 2 == 0 and UL % 2 == 0

    def attn_block(u0, nu, m_cur, m8, last):
        ms = {0: m_cur}
        acc = None
        for i in range(nu * NC):
            gi = L + i
            su, sc = gi // NC, gi % NC
            pu, pc = i // NC, i % NC

            def s_part():
                nonlocal m8
                if not (last and su >= nu):
                    m8 = s1_chunk(u0 + su, sc, gi % RS, m8 if sc > 0 else None)
                    if sc == NC - 1:
                        ms[su] = jnp.max(m8, axis=0, keepdims=True)

            def p_part():
                nonlocal acc
                acc = s2_chunk(pc, i % RS, ms[pu], acc if pc > 0 else None)
                if pc == NC - 1:
                    finish(u0 + pu, acc)
            if ORDER == 0:
                s_part(); p_part()
            else:
                p_part(); s_part()
        if last:
            return None
        return ms[nu], m8

    def attn_phase():
        m8 = None
        m0 = None
        for gi in range(L):
            su, sc = gi // NC, gi % NC
            m8 = s1_chunk(su, sc, gi % RS, m8 if sc > 0 else None)
            if sc == NC - 1:
                m0 = jnp.max(m8, axis=0, keepdims=True)
        c = jax.lax.fori_loop(0, NI, lambda t, c: attn_block(t * U, U, c[0], c[1], False), (m0, m8))
        attn_block(NI * U, UL, c[0], c[1], True)

    def ocopy(b):
        return pltpu.make_async_copy(obuf_ref.at[b], out_hbm.at[0, :, pl.ds(pl.multiple_of(b * TQ, TQ), TQ)], sem_out.at[b])

    def ffn_phase(final):
        def body(b, c):
            a = jnp.dot(woT_ref[...], oT_ref[b], preferred_element_type=F32)
            x1 = xT_ref[b] + a
            xn = _ln(x1).astype(BF16)
            y = x1
            for f in range(DFF // FC):
                hc = jnp.dot(w1T_ref[f * FC:(f + 1) * FC, :], xn, preferred_element_type=F32)
                hc = jnp.maximum(hc, 0.0).astype(BF16)
                y = y + jnp.dot(w2T_ref[:, f * FC:(f + 1) * FC], hc, preferred_element_type=F32)
            if final:
                obuf_ref[b] = y.astype(BF16)
                ocopy(b).start()
            else:
                xT_ref[b] = y
                proj(b, y)
            return c
        jax.lax.fori_loop(0, NQB, body, 0)

    def layer(l, c):
        attn_phase()

        @pl.when(l == 0)
        def _():
            wcopies[5].wait()
            ffn_phase(False)

        @pl.when(l == 1)
        def _():
            ffn_phase(True)
        return c
    jax.lax.fori_loop(0, 2, layer, 0)

    for b in range(NQB):
        ocopy(b).wait()


@jax.jit
def pallas_interleave_layers__grouped_kv_mqa__dense_activation_relu__prompt_kernel(A_x, A_wq, A_wk, A_wv, A_wo, B_x, B_w1, B_w2):
    hbm = pl.BlockSpec(memory_space=pltpu.HBM)
    scratch = [
        pltpu.VMEM((NQB, D, TQ), BF16),
        pltpu.VMEM((D, D), BF16),
        pltpu.VMEM((DH, D), BF16),
        pltpu.VMEM((DH, D), BF16),
        pltpu.VMEM((D, D), BF16),
        pltpu.VMEM((D, DFF), BF16),
        pltpu.VMEM((QKVR, D), BF16),
        pltpu.VMEM((D, H * HP), BF16),
        pltpu.VMEM((DFF, D), BF16),
        pltpu.VMEM((D, DFF), BF16),
        pltpu.VMEM((H * HP, D), F32),
        pltpu.VMEM((NQB, D, TQ), F32),
        pltpu.VMEM((NQB, H * HP, TQ), BF16),
        pltpu.VMEM((S, HP), BF16),
        pltpu.VMEM((NQB, HP, TQ), BF16),
        pltpu.VMEM((NQB, H * HP, TQ), BF16),
        pltpu.VMEM((2 * S, TQ), F32),
        pltpu.VMEM((NQB, D, TQ), BF16),
        pltpu.SemaphoreType.DMA((NQB + 6,)),
        pltpu.SemaphoreType.DMA((NQB,)),
    ]
    outT = pl.pallas_call(
        _kernel,
        out_shape=jax.ShapeDtypeStruct((1, D, S), BF16),
        in_specs=[hbm] * 7,
        out_specs=hbm,
        scratch_shapes=scratch,
        compiler_params=pltpu.CompilerParams(vmem_limit_bytes=100 * 1024 * 1024),
    )(jnp.transpose(A_x, (0, 2, 1)), A_wq, A_wk.T, A_wv.T, A_wo, B_w1, B_w2.T)
    return jnp.transpose(outT, (0, 2, 1))
```

```python
import functools

import jax
import jax.numpy as jnp
import jax.experimental.pallas as pl
import jax.experimental.pallas.tpu as pltpu

F32 = jnp.float32
BF16 = jnp.bfloat16

S = 2048
D = 448
H = 16
DH = 28
HP = 32
DFF = 1792
TQ = 512
NQB = S // TQ
CK = 128
NC = S // CK
U = 6
UL = 4
ORDER = 1
SKEW = 4
FC = 256
EPS = 1e-5
KROW = 0
VROW = HP
QROW = 2 * HP
QKVR = D + 2 * HP
QSCALE = (DH ** -0.5) * 1.4426950408889634


def _ln(x):
    m = jnp.mean(x, axis=0, keepdims=True)
    xc = x - m
    v = jnp.mean(xc * xc, axis=0, keepdims=True)
    return xc * jax.lax.rsqrt(v + EPS)


def _kernel(x_hbm, wq_hbm, wk_hbm, wv_hbm, wo_hbm, w1_hbm, w2_hbm, out_hbm,
            xin_ref, wq_ref, wk_ref, wv_ref, wo_ref, w1_ref,
            wqkvT_ref, woT_ref, w1T_ref, w2T_ref, tmp_ref,
            xT_ref, qT_ref, k_ref, vT_ref, oT_ref, s_ref, obuf_ref,
            sem_in, sem_out):
    def xcopy(b):
        off = b * TQ if isinstance(b, int) else pl.multiple_of(b * TQ, TQ)
        return pltpu.make_async_copy(x_hbm.at[0, :, pl.ds(off, TQ)], xin_ref.at[b], sem_in.at[b])
    wcopies = [pltpu.make_async_copy(src, dst, sem_in.at[NQB + i])
               for i, (src, dst) in enumerate([(wq_hbm, wq_ref), (wk_hbm, wk_ref), (wv_hbm, wv_ref),
                                               (wo_hbm, wo_ref), (w1_hbm, w1_ref), (w2_hbm, w2T_ref)])]
    for i in range(3):
        wcopies[i].start()
    for b in range(NQB):
        xcopy(b).start()
    for i in range(3, 6):
        wcopies[i].start()

    def proj_mm(b, xn):
        qkv = jnp.dot(wqkvT_ref[...], xn, preferred_element_type=F32)
        q = jnp.concatenate([qkv[QROW + h * DH:QROW + h * DH + HP] for h in range(H - 1)]
                            + [qkv[QROW + (H - 1) * DH:QROW + H * DH], qkv[QROW:QROW + HP - DH]], axis=0)
        qT_ref[b] = (q * QSCALE).astype(BF16)
        kT = qkv[KROW:KROW + HP].T.astype(BF16)
        if isinstance(b, int):
            k_ref[b * TQ:(b + 1) * TQ, :] = kT
        else:
            k_ref[pl.ds(pl.multiple_of(b * TQ, TQ), TQ), :] = kT
        v = qkv[VROW:VROW + HP]
        row = jax.lax.broadcasted_iota(jnp.int32, v.shape, 0)
        vT_ref[b] = jnp.where(row == DH, 1.0, v).astype(BF16)

    def proj(b, x):
        proj_mm(b, _ln(x).astype(BF16))

    wcopies[0].wait(); wcopies[1].wait(); wcopies[2].wait()
    wqkvT_ref[QROW:QROW + D, :] = wq_ref[...].T
    kv = jnp.concatenate([wk_ref[...].astype(F32), jnp.zeros((HP - DH, D), F32),
                          wv_ref[...].astype(F32), jnp.zeros((HP - DH, D), F32)], axis=0)
    wqkvT_ref[KROW:KROW + 2 * HP, :] = kv.astype(BF16)

    def proj0(b):
        x = xin_ref[b].astype(F32)
        xT_ref[b] = x
        proj(b, x)

    xcopy(0).wait()
    proj0(0)
    for b in range(1, NQB):
        xcopy(b).wait()
    for b in range(1, NQB):
        proj0(b)
    wcopies[3].wait(); wcopies[4].wait()

    def weight_prep():
        tmp_ref[...] = jnp.zeros((H * HP, D), F32)
        wo32 = wo_ref[...].astype(F32)
        for h in range(H):
            tmp_ref[h * HP:h * HP + DH, :] = wo32[h * DH:(h + 1) * DH, :]
        woT_ref[...] = tmp_ref[...].T.astype(BF16)
        w1T_ref[...] = w1_ref[...].T

    def s1_chunk(u, c, slot, m8):
        h = u & 15; qb = u >> 4
        if isinstance(u, int):
            qblk = qT_ref[qb, h * HP:(h + 1) * HP, :]
        else:
            qblk = qT_ref[qb, pl.ds(pl.multiple_of(h * HP, HP), HP), :]
        kblk = k_ref[c * CK:(c + 1) * CK, :]
        s = jnp.dot(kblk, qblk, preferred_element_type=F32)
        s_ref[slot * CK:(slot + 1) * CK, :] = s
        mm = jnp.max(s.reshape(CK // 8, 8, TQ), axis=0)
        return mm if m8 is None else jnp.maximum(m8, mm)

    def s2_chunk(c, slot, m, acc):
        p = jnp.exp2(s_ref[slot * CK:(slot + 1) * CK, :] - m).astype(BF16)
        per = TQ // CK
        vblk = vT_ref[c // per, :, (c % per) * CK:(c % per + 1) * CK]
        o = jnp.dot(vblk, p, preferred_element_type=F32)
        return o if acc is None else acc + o

    def finish(u, acc):
        h = u & 15; qb = u >> 4
        o = (acc * (1.0 / acc[DH:DH + 1, :])).astype(BF16)
        if isinstance(u, int):
            oT_ref[qb, h * HP:(h + 1) * HP, :] = o
        else:
            oT_ref[qb, pl.ds(pl.multiple_of(h * HP, HP), HP), :] = o

    RS = 2 * NC
    L = NC + SKEW
    NU = H * NQB
    NI = (NU - UL) // U
    assert U * NI + UL == NU and U % 2 == 0 and UL % 2 == 0

    def attn_block(u0, nu, m_cur, m8, last):
        ms = {0: m_cur}
        acc = None
        for i in range(nu * NC):
            gi = L + i
            su, sc = gi // NC, gi % NC
            pu, pc = i // NC, i % NC

            def s_part():
                nonlocal m8
                if not (last and su >= nu):
                    m8 = s1_chunk(u0 + su, sc, gi % RS, m8 if sc > 0 else None)
                    if sc == NC - 1:
                        ms[su] = jnp.max(m8, axis=0, keepdims=True)

            def p_part():
                nonlocal acc
                acc = s2_chunk(pc, i % RS, ms[pu], acc if pc > 0 else None)
                if pc == NC - 1:
                    finish(u0 + pu, acc)
            if ORDER == 0:
                s_part(); p_part()
            else:
                p_part(); s_part()
        if last:
            return None
        return ms[nu], m8

    def attn_phase():
        weight_prep()
        m8 = None
        m0 = None
        for gi in range(L):
            su, sc = gi // NC, gi % NC
            m8 = s1_chunk(su, sc, gi % RS, m8 if sc > 0 else None)
            if sc == NC - 1:
                m0 = jnp.max(m8, axis=0, keepdims=True)
        c = jax.lax.fori_loop(0, NI, lambda t, c: attn_block(t * U, U, c[0], c[1], False), (m0, m8))
        attn_block(NI * U, UL, c[0], c[1], True)

    def ocopy(b):
        return pltpu.make_async_copy(obuf_ref.at[b], out_hbm.at[0, :, pl.ds(pl.multiple_of(b * TQ, TQ), TQ)], sem_out.at[b])

    def ffn_phase(final):
        def body(b, c):
            a = jnp.dot(woT_ref[...], oT_ref[b], preferred_element_type=F32)
            x1 = xT_ref[b] + a
            xn = _ln(x1).astype(BF16)
            y = x1
            for f in range(DFF // FC):
                hc = jnp.dot(w1T_ref[f * FC:(f + 1) * FC, :], xn, preferred_element_type=F32)
                hc = jnp.maximum(hc, 0.0).astype(BF16)
                y = y + jnp.dot(w2T_ref[:, f * FC:(f + 1) * FC], hc, preferred_element_type=F32)
            if final:
                obuf_ref[b] = y.astype(BF16)
                ocopy(b).start()
            else:
                xT_ref[b] = y
                proj(b, y)
            return c
        jax.lax.fori_loop(0, NQB, body, 0)

    def layer(l, c):
        attn_phase()

        @pl.when(l == 0)
        def _():
            wcopies[5].wait()
            ffn_phase(False)

        @pl.when(l == 1)
        def _():
            ffn_phase(True)
        return c
    jax.lax.fori_loop(0, 2, layer, 0)

    for b in range(NQB):
        ocopy(b).wait()


@jax.jit
def pallas_interleave_layers__grouped_kv_mqa__dense_activation_relu__prompt_kernel(A_x, A_wq, A_wk, A_wv, A_wo, B_x, B_w1, B_w2):
    hbm = pl.BlockSpec(memory_space=pltpu.HBM)
    scratch = [
        pltpu.VMEM((NQB, D, TQ), BF16),
        pltpu.VMEM((D, D), BF16),
        pltpu.VMEM((DH, D), BF16),
        pltpu.VMEM((DH, D), BF16),
        pltpu.VMEM((D, D), BF16),
        pltpu.VMEM((D, DFF), BF16),
        pltpu.VMEM((QKVR, D), BF16),
        pltpu.VMEM((D, H * HP), BF16),
        pltpu.VMEM((DFF, D), BF16),
        pltpu.VMEM((D, DFF), BF16),
        pltpu.VMEM((H * HP, D), F32),
        pltpu.VMEM((NQB, D, TQ), F32),
        pltpu.VMEM((NQB, H * HP, TQ), BF16),
        pltpu.VMEM((S, HP), BF16),
        pltpu.VMEM((NQB, HP, TQ), BF16),
        pltpu.VMEM((NQB, H * HP, TQ), BF16),
        pltpu.VMEM((2 * S, TQ), F32),
        pltpu.VMEM((NQB, D, TQ), BF16),
        pltpu.SemaphoreType.DMA((NQB + 6,)),
        pltpu.SemaphoreType.DMA((NQB,)),
    ]
    outT = pl.pallas_call(
        _kernel,
        out_shape=jax.ShapeDtypeStruct((1, D, S), BF16),
        in_specs=[hbm] * 7,
        out_specs=hbm,
        scratch_shapes=scratch,
        compiler_params=pltpu.CompilerParams(vmem_limit_bytes=100 * 1024 * 1024),
    )(jnp.transpose(A_x, (0, 2, 1)), A_wq, A_wk.T, A_wv.T, A_wo, B_w1, B_w2.T)
    return jnp.transpose(outT, (0, 2, 1))
```

```python
import jax
import jax.numpy as jnp
import jax.experimental.pallas as pl
import jax.experimental.pallas.tpu as pltpu

F32 = jnp.float32
BF16 = jnp.bfloat16

S = 2048
D = 448
H = 16
DH = 28
HP = 32
DFF = 1792
TQ = 512
NQB = S // TQ
CK = 128
NC = S // CK
U = 6
UL = 4
SKEW = 4
FC = 256
EPS = 1e-5
KROW = 0
VROW = HP
QROW = 2 * HP
QKVR = D + 2 * HP
QSCALE = (DH ** -0.5) * 1.4426950408889634


def _ln(x):
    m = jnp.mean(x, axis=0, keepdims=True)
    xc = x - m
    v = jnp.mean(xc * xc, axis=0, keepdims=True)
    return xc * jax.lax.rsqrt(v + EPS)


def _kernel(x_hbm, wq_hbm, wk_hbm, wv_hbm, wo_hbm, w1_hbm, w2_hbm, out_hbm,
            xin_ref, wq_ref, wk_ref, wv_ref, wo_ref, w1_ref,
            wqkvT_ref, woT_ref, w1T_ref, w2T_ref, tmp_ref,
            xT_ref, qT_ref, k_ref, vT_ref, oT_ref, s_ref, obuf_ref,
            sem_in, sem_out):
    def xcopy(b):
        return pltpu.make_async_copy(x_hbm.at[0, :, pl.ds(b * TQ, TQ)], xin_ref.at[b], sem_in.at[b])
    wcopies = [pltpu.make_async_copy(src, dst, sem_in.at[NQB + i])
               for i, (src, dst) in enumerate([(wq_hbm, wq_ref), (wk_hbm, wk_ref), (wv_hbm, wv_ref),
                                               (wo_hbm, wo_ref), (w1_hbm, w1_ref), (w2_hbm, w2T_ref)])]
    for i in range(3):
        wcopies[i].start()
    for b in range(NQB):
        xcopy(b).start()
    for i in range(3, 6):
        wcopies[i].start()

    def proj(b, x):
        xn = _ln(x).astype(BF16)
        qkv = jnp.dot(wqkvT_ref[...], xn, preferred_element_type=F32)
        q = jnp.concatenate([qkv[QROW + h * DH:QROW + h * DH + HP] for h in range(H - 1)]
                            + [qkv[QROW + (H - 1) * DH:QROW + H * DH], qkv[QROW:QROW + HP - DH]], axis=0)
        qT_ref[b] = (q * QSCALE).astype(BF16)
        kT = qkv[KROW:KROW + HP].T.astype(BF16)
        if isinstance(b, int):
            k_ref[b * TQ:(b + 1) * TQ, :] = kT
        else:
            k_ref[pl.ds(pl.multiple_of(b * TQ, TQ), TQ), :] = kT
        v = qkv[VROW:VROW + HP]
        row = jax.lax.broadcasted_iota(jnp.int32, v.shape, 0)
        vT_ref[b] = jnp.where(row == DH, 1.0, v).astype(BF16)

    wcopies[0].wait(); wcopies[1].wait(); wcopies[2].wait()
    wqkvT_ref[QROW:QROW + D, :] = wq_ref[...].T
    kv = jnp.concatenate([wk_ref[...].astype(F32), jnp.zeros((HP - DH, D), F32),
                          wv_ref[...].astype(F32), jnp.zeros((HP - DH, D), F32)], axis=0)
    wqkvT_ref[KROW:KROW + 2 * HP, :] = kv.astype(BF16)

    def proj0(b):
        x = xin_ref[b].astype(F32)
        xT_ref[b] = x
        proj(b, x)

    xcopy(0).wait()
    proj0(0)
    for b in range(1, NQB):
        xcopy(b).wait()
    for b in range(1, NQB):
        proj0(b)
    wcopies[3].wait(); wcopies[4].wait()

    def weight_prep():
        tmp_ref[...] = jnp.zeros((H * HP, D), F32)
        wo32 = wo_ref[...].astype(F32)
        for h in range(H):
            tmp_ref[h * HP:h * HP + DH, :] = wo32[h * DH:(h + 1) * DH, :]
        woT_ref[...] = tmp_ref[...].T.astype(BF16)
        w1T_ref[...] = w1_ref[...].T

    def score_chunk(u, c, slot, m8):
        h = u & 15; qb = u >> 4
        if isinstance(u, int):
            qblk = qT_ref[qb, h * HP:(h + 1) * HP, :]
        else:
            qblk = qT_ref[qb, pl.ds(pl.multiple_of(h * HP, HP), HP), :]
        kblk = k_ref[c * CK:(c + 1) * CK, :]
        s = jnp.dot(kblk, qblk, preferred_element_type=F32)
        s_ref[slot * CK:(slot + 1) * CK, :] = s
        mm = jnp.max(s.reshape(CK // 8, 8, TQ), axis=0)
        return mm if m8 is None else jnp.maximum(m8, mm)

    def pv_chunk(c, slot, m, acc):
        p = jnp.exp2(s_ref[slot * CK:(slot + 1) * CK, :] - m).astype(BF16)
        per = TQ // CK
        vblk = vT_ref[c // per, :, (c % per) * CK:(c % per + 1) * CK]
        o = jnp.dot(vblk, p, preferred_element_type=F32)
        return o if acc is None else acc + o

    def finish(u, acc):
        h = u & 15; qb = u >> 4
        o = (acc * (1.0 / acc[DH:DH + 1, :])).astype(BF16)
        if isinstance(u, int):
            oT_ref[qb, h * HP:(h + 1) * HP, :] = o
        else:
            oT_ref[qb, pl.ds(pl.multiple_of(h * HP, HP), HP), :] = o

    RS = 2 * NC
    L = NC + SKEW
    NU = H * NQB
    NI = (NU - UL) // U
    assert U * NI + UL == NU and U % 2 == 0 and UL % 2 == 0 and L < RS and L <= UL * NC

    def attn_block(u0, nu, m_cur, m8, last):
        ms = {0: m_cur}
        acc = None
        for i in range(nu * NC):
            gi = L + i
            su, sc = gi // NC, gi % NC
            pu, pc = i // NC, i % NC
            acc = pv_chunk(pc, i % RS, ms[pu], acc if pc > 0 else None)
            if pc == NC - 1:
                finish(u0 + pu, acc)
            if not (last and su >= nu):
                m8 = score_chunk(u0 + su, sc, gi % RS, m8 if sc > 0 else None)
                if sc == NC - 1:
                    ms[su] = jnp.max(m8, axis=0, keepdims=True)
        if last:
            return None
        return ms[nu], m8

    def attn_phase():
        weight_prep()
        m8 = None
        m0 = None
        for gi in range(L):
            su, sc = gi // NC, gi % NC
            m8 = score_chunk(su, sc, gi % RS, m8 if sc > 0 else None)
            if sc == NC - 1:
                m0 = jnp.max(m8, axis=0, keepdims=True)
        c = jax.lax.fori_loop(0, NI, lambda t, c: attn_block(t * U, U, c[0], c[1], False), (m0, m8))
        attn_block(NI * U, UL, c[0], c[1], True)

    def ocopy(b):
        off = b * TQ if isinstance(b, int) else pl.multiple_of(b * TQ, TQ)
        return pltpu.make_async_copy(obuf_ref.at[b], out_hbm.at[0, :, pl.ds(off, TQ)], sem_out.at[b])

    def ffn_phase(final):
        def body(b, c):
            a = jnp.dot(woT_ref[...], oT_ref[b], preferred_element_type=F32)
            x1 = xT_ref[b] + a
            xn = _ln(x1).astype(BF16)
            y = x1
            for f in range(DFF // FC):
                hc = jnp.dot(w1T_ref[f * FC:(f + 1) * FC, :], xn, preferred_element_type=F32)
                hc = jnp.maximum(hc, 0.0).astype(BF16)
                y = y + jnp.dot(w2T_ref[:, f * FC:(f + 1) * FC], hc, preferred_element_type=F32)
            if final:
                obuf_ref[b] = y.astype(BF16)
                ocopy(b).start()
            else:
                xT_ref[b] = y
                proj(b, y)
            return c
        jax.lax.fori_loop(0, NQB, body, 0)

    def layer(l, c):
        attn_phase()

        @pl.when(l == 0)
        def _():
            wcopies[5].wait()
            ffn_phase(False)

        @pl.when(l == 1)
        def _():
            ffn_phase(True)
        return c
    jax.lax.fori_loop(0, 2, layer, 0)

    for b in range(NQB):
        ocopy(b).wait()


@jax.jit
def pallas_interleave_layers__grouped_kv_mqa__dense_activation_relu__prompt_kernel(A_x, A_wq, A_wk, A_wv, A_wo, B_x, B_w1, B_w2):
    hbm = pl.BlockSpec(memory_space=pltpu.HBM)
    scratch = [
        pltpu.VMEM((NQB, D, TQ), BF16),
        pltpu.VMEM((D, D), BF16),
        pltpu.VMEM((DH, D), BF16),
        pltpu.VMEM((DH, D), BF16),
        pltpu.VMEM((D, D), BF16),
        pltpu.VMEM((D, DFF), BF16),
        pltpu.VMEM((QKVR, D), BF16),
        pltpu.VMEM((D, H * HP), BF16),
        pltpu.VMEM((DFF, D), BF16),
        pltpu.VMEM((D, DFF), BF16),
        pltpu.VMEM((H * HP, D), F32),
        pltpu.VMEM((NQB, D, TQ), F32),
        pltpu.VMEM((NQB, H * HP, TQ), BF16),
        pltpu.VMEM((S, HP), BF16),
        pltpu.VMEM((NQB, HP, TQ), BF16),
        pltpu.VMEM((NQB, H * HP, TQ), BF16),
        pltpu.VMEM((2 * S, TQ), F32),
        pltpu.VMEM((NQB, D, TQ), BF16),
        pltpu.SemaphoreType.DMA((NQB + 6,)),
        pltpu.SemaphoreType.DMA((NQB,)),
    ]
    outT = pl.pallas_call(
        _kernel,
        out_shape=jax.ShapeDtypeStruct((1, D, S), BF16),
        in_specs=[hbm] * 7,
        out_specs=hbm,
        scratch_shapes=scratch,
        compiler_params=pltpu.CompilerParams(vmem_limit_bytes=100 * 1024 * 1024),
    )(jnp.transpose(A_x, (0, 2, 1)), A_wq, A_wk.T, A_wv.T, A_wo, B_w1, B_w2.T)
    return jnp.transpose(outT, (0, 2, 1))
```
